```python
import jax
import jax.numpy as jnp

def _softmax(x, axis=-1):
    return jax.nn.softmax(x, axis=axis)

def _gelu(x):
    return jax.nn.gelu(x, approximate=True)

def _silu(x):
    return jax.nn.silu(x)

def _sigmoid(x):
    return jax.nn.sigmoid(x)

def _layernorm(x, axis=-1, eps=1e-05):
    m = jnp.mean(x, axis=axis, keepdims=True)
    v = jnp.var(x, axis=axis, keepdims=True)
    return (x - m) / jnp.sqrt(v + eps)

def _scatter_add(tgt, idx, src, axis=0):
    return tgt.at[idx].add(src)

def _segment_sum(src, seg, n):
    return jax.ops.segment_sum(src, seg, n)

class _Rng:

    def __init__(self, key):
        self._k = key

    def _next(self):
        self._k, sub = jax.random.split(self._k)
        return sub

    def normal(self, shape):
        return jax.random.normal(self._next(), shape, dtype=jnp.bfloat16)

    def randint(self, lo, hi, shape):
        return jax.random.randint(self._next(), shape, lo, hi, dtype=jnp.int32)

    def uniform(self, shape, lo=0.0, hi=1.0):
        return jax.random.uniform(self._next(), shape, jnp.bfloat16, lo, hi)

    def permutation(self, n):
        return jax.random.permutation(self._next(), n)
kernel_name = 'adaLN_cond__sliding_block_cached__mixer_s_mlp__decode'

def setup_inputs():
    _rng = _Rng(jax.random.key(int.from_bytes(__import__("os").urandom(4), "little")))
    _w = lambda a: (lambda t: t.astype(jnp.bfloat16) if jnp.issubdtype(t.dtype, jnp.floating) else t)(jnp.asarray(a))

    def _A_setup():
        B, Sq, D = (1, 1, 448)
        Hq, Hkv, Sk, Dh = (16, 8, 65536, 256)
        assert Hq % Hkv == 0, (Hq, Hkv)
        return {'x': _w((lambda *s: _rng.normal(s) * 0.05)(B, Sq, D)), 'k_cache': _w((lambda *s: _rng.normal(s) * 0.05)(B, Hkv, Sk, Dh)), 'v_cache': _w((lambda *s: _rng.normal(s) * 0.05)(B, Hkv, Sk, Dh)), 'wq': _w((lambda *s: _rng.normal(s) * 0.05)(D, Hq * Dh) * D ** (-0.5)), 'wo': _w((lambda *s: _rng.normal(s) * 0.05)(Hq * Dh, D) * (Hq * Dh) ** (-0.5))}
    _A_in = _A_setup()

    def _B_setup():
        B, S, D, F = (1, 1, 448, 1792)
        return {'x': _w((lambda *s: _rng.normal(s) * 0.05)(B, S, D)), 'w1': _w((lambda *s: _rng.normal(s) * 0.05)(D, D) * D ** (-0.5)), 'w2': _w((lambda *s: _rng.normal(s) * 0.05)(D, D) * D ** (-0.5)), 'w3': _w((lambda *s: _rng.normal(s) * 0.05)(D, F) * D ** (-0.5)), 'w4': _w((lambda *s: _rng.normal(s) * 0.05)(F, D) * F ** (-0.5))}
    _B_in = _B_setup()
    return {'A_x': _A_in['x'], 'A_k_cache': _A_in['k_cache'], 'A_v_cache': _A_in['v_cache'], 'A_wq': _A_in['wq'], 'A_wo': _A_in['wo'], 'B_x': _B_in['x'], 'B_w1': _B_in['w1'], 'B_w2': _B_in['w2'], 'B_w3': _B_in['w3'], 'B_w4': _B_in['w4'], 'c': _w((lambda *s: _rng.normal(s) * 0.05)(1, 448)), 'w_mod': _w((lambda *s: _rng.normal(s) * 0.05)(448, 6 * 448) * 448 ** (-0.5))}

def reference(A_x, A_k_cache, A_v_cache, A_wq, A_wo, B_x, B_w1, B_w2, B_w3, B_w4, c, w_mod):

    def _A_ref(x, k_cache, v_cache, wq, wo):
        B, Sq, D = x.shape
        Hq, Dh = (16, 256)
        Hkv, Sk = (k_cache.shape[1], k_cache.shape[2])
        W = min(4096, max(256, Sk // 4))
        rep = Hq // Hkv
        q = (lambda x, *d: x.transpose(*d))((x @ wq).reshape(B, Sq, Hq, Dh), 0, 2, 1, 3)
        k = jnp.repeat(k_cache[:, :, Sk - W:, :], rep, axis=1)
        v = jnp.repeat(v_cache[:, :, Sk - W:, :], rep, axis=1)
        scores = jnp.einsum('bhqd,bhkd->bhqk', q, k) * Dh ** (-0.5)
        p = _softmax(scores, axis=-1)
        o = jnp.einsum('bhqk,bhkd->bhqd', p, v)
        return (lambda x, *d: x.transpose(*d))(o, 0, 2, 1, 3).reshape(B, Sq, Hq * Dh) @ wo

    def _B_ref(x, w1, w2, w3, w4):
        B, S, D = x.shape
        h = _gelu(_layernorm(x, axis=-1) @ w1)
        c = D // 4
        g0 = jnp.pad(h[:, :, 0 * c:1 * c], ((0, 0), (1, 0), (0, 0)))[:, :S, :]
        g1 = jnp.pad(h[:, :, 1 * c:2 * c], ((0, 0), (0, 1), (0, 0)))[:, 1:, :]
        g2 = jnp.pad(h[:, :, 2 * c:3 * c], ((0, 0), (2, 0), (0, 0)))[:, :S, :]
        g3 = jnp.pad(h[:, :, 3 * c:], ((0, 0), (0, 2), (0, 0)))[:, 2:, :]
        hs = jnp.concatenate([g0, g1, g2, g3], axis=-1) @ w2
        x1 = x + hs
        h2 = _gelu(_layernorm(x1, axis=-1) @ w3) @ w4
        return x1 + h2
    x = A_x
    mod = (_silu(c) @ w_mod).reshape(c.shape[0], 6, 1, -1)
    sa, ca, ga, sb, cb, gb = (mod[:, 0].copy(), mod[:, 1].copy(), mod[:, 2].copy(), mod[:, 3].copy(), mod[:, 4].copy(), mod[:, 5].copy())
    h = _layernorm(x, axis=-1) * (1 + ca) + sa
    x = x + ga * _A_ref(h, A_k_cache, A_v_cache, A_wq, A_wo)
    h = _layernorm(x, axis=-1) * (1 + cb) + sb
    x = x + gb * _B_ref(h, B_w1, B_w2, B_w3, B_w4)
    return x
```

```python
import jax
import jax.numpy as jnp
import jax.experimental.pallas as pl
import jax.experimental.pallas.tpu as pltpu

D = 448
F = 1792
HQ = 16
HKV = 8
DH = 256
EPS = 1e-5
ROWS = 8
W4_SPLIT = (11, 3)

_NT = (((1,), (1,)), ((), ()))
bf16 = jnp.bfloat16
f32 = jnp.float32


def _layernorm(x):
    m = jnp.mean(x, axis=-1, keepdims=True)
    d = x - m
    v = jnp.mean(d * d, axis=-1, keepdims=True)
    return d * jax.lax.rsqrt(v + EPS)


def _kernel(x_hbm, k_hbm, v_hbm, wq_hbm, wot_hbm, w3_hbm, w4t_hbm, c_hbm, wm_hbm, o_ref,
            x_buf, c_buf, wm_buf, wq_buf, k_buf, v_buf, wot_buf, w3_buf, w4t_buf,
            qo_buf, p_buf, sems):
    window = k_buf.shape[1]
    win = pl.ds(k_hbm.shape[2] - window, window)
    copies = {}

    def start(name, src, dst):
        copies[name] = pltpu.make_async_copy(src, dst, sems.at[len(copies)])
        copies[name].start()

    start("wm", wm_hbm, wm_buf)
    start("x", x_hbm, x_buf)
    start("c", c_hbm, c_buf)
    start("wq", wq_hbm, wq_buf)
    start("k", k_hbm.at[0, :, win, :], k_buf)
    start("v", v_hbm.at[0, :, win, :], v_buf)
    start("wo", wot_hbm, wot_buf)
    start("w3", w3_hbm, w3_buf)
    w4_cols, f0 = [], 0
    for i, n in enumerate(W4_SPLIT):
        cols = pl.ds(f0, n * 128)
        start(("w4", i), w4t_hbm.at[:, cols], w4t_buf.at[:, cols])
        w4_cols.append((f0, f0 + n * 128))
        f0 += n * 128

    copies["wm"].wait()
    copies["x"].wait()
    copies["c"].wait()
    c = jnp.broadcast_to(c_buf[...].astype(f32), (ROWS, D))
    s = (c * jax.nn.sigmoid(c)).astype(bf16)
    x = jnp.broadcast_to(x_buf[0].astype(f32), (ROWS, D))
    mod = jnp.dot(s, wm_buf[...], preferred_element_type=f32)
    sa, ca, ga, sb, cb, gb = [mod[:, i * D:(i + 1) * D] for i in range(6)]
    h = (_layernorm(x) * (1.0 + ca) + sa).astype(bf16)

    copies["wq"].wait()
    q = jnp.dot(h, wq_buf[...], preferred_element_type=f32)
    even = jax.lax.broadcasted_iota(jnp.int32, (ROWS, DH), 0) % 2 == 0
    for j in range(HKV):
        lo = 2 * j * DH
        qo_buf[j] = jnp.where(even, q[:, lo:lo + DH], q[:, lo + DH:lo + 2 * DH])

    copies["k"].wait()

    def probs(j, carry):
        sc = jax.lax.dot_general(qo_buf[j].astype(bf16), k_buf[j], _NT,
                                 preferred_element_type=f32) * (DH ** -0.5)
        p = jnp.exp(sc - jnp.max(sc, axis=-1, keepdims=True))
        p_buf[j] = p * (1.0 / jnp.sum(p, axis=-1, keepdims=True))
        return carry

    jax.lax.fori_loop(0, HKV, probs, None)

    copies["v"].wait()

    def values(j, carry):
        qo_buf[j] = jnp.dot(p_buf[j].astype(bf16), v_buf[j], preferred_element_type=f32)
        return carry

    jax.lax.fori_loop(0, HKV, values, None)

    copies["wo"].wait()
    parts = []
    for j in range(HKV):
        o = qo_buf[j]
        parts += [jnp.where(even, o, 0.0), jnp.where(even, 0.0, o)]
    o = jnp.concatenate(parts, axis=1).astype(bf16)
    a = jax.lax.dot_general(o, wot_buf[...], _NT, preferred_element_type=f32)
    a = a + pltpu.roll(a, 1, 0)
    x2 = x + ga * a
    x1 = _layernorm(x2) * (1.0 + cb) + sb
    h3 = _layernorm(x1).astype(bf16)

    copies["w3"].wait()
    g = jnp.dot(h3, w3_buf[...], preferred_element_type=f32)
    g = jax.nn.gelu(g, approximate=True).astype(bf16)
    acc = x2 + gb * x1
    for i, (lo, hi) in enumerate(w4_cols):
        copies["w4", i].wait()
        acc = acc + gb * jax.lax.dot_general(g[:, lo:hi], w4t_buf[:, lo:hi], _NT,
                                             preferred_element_type=f32)
    o_ref[0] = acc[0:1].astype(o_ref.dtype)


@jax.jit
def pallas_adaLN_cond__sliding_block_cached__mixer_s_mlp__decode_kernel(
    A_x: jax.Array,
    A_k_cache: jax.Array,
    A_v_cache: jax.Array,
    A_wq: jax.Array,
    A_wo: jax.Array,
    B_x: jax.Array,
    B_w1: jax.Array,
    B_w2: jax.Array,
    B_w3: jax.Array,
    B_w4: jax.Array,
    c: jax.Array,
    w_mod: jax.Array,
):
    assert A_x.shape == (1, 1, D) and A_k_cache.shape[:2] == (1, HKV)
    window = min(4096, max(256, A_k_cache.shape[2] // 4))
    hbm = pl.BlockSpec(memory_space=pltpu.HBM)
    return pl.pallas_call(
        _kernel,
        out_shape=jax.ShapeDtypeStruct(A_x.shape, A_x.dtype),
        in_specs=[hbm] * 9,
        scratch_shapes=[
            pltpu.VMEM((1, 1, D), bf16),
            pltpu.VMEM((1, D), bf16),
            pltpu.VMEM((D, 6 * D), bf16),
            pltpu.VMEM((D, HQ * DH), bf16),
            pltpu.VMEM((HKV, window, DH), bf16),
            pltpu.VMEM((HKV, window, DH), bf16),
            pltpu.VMEM((D, HQ * DH), bf16),
            pltpu.VMEM((D, F), bf16),
            pltpu.VMEM((D, F), bf16),
            pltpu.VMEM((HKV, ROWS, DH), f32),
            pltpu.VMEM((HKV, ROWS, window), f32),
            pltpu.SemaphoreType.DMA((8 + len(W4_SPLIT),)),
        ],
        compiler_params=pltpu.CompilerParams(
            vmem_limit_bytes=100 * 2**20,
            disable_bounds_checks=True,
            disable_semaphore_checks=True,
        ),
    )(A_x, A_k_cache, A_v_cache, A_wq, A_wo.T, B_w3, B_w4.T, c, w_mod)
```

```python
import jax
import jax.numpy as jnp
import jax.experimental.pallas as pl
import jax.experimental.pallas.tpu as pltpu

D = 448
F = 1792
HQ = 16
HKV = 8
DH = 256
EPS = 1e-5
SUB = 8
LANE = 128

W4_MXU_ROWS = 256
W4_VPU_ROWS = (96, 56, 32, 8)
W4_VPU_DEFERRED = 2

_NT = (((1,), (1,)), ((), ()))
bf16 = jnp.bfloat16
f32 = jnp.float32


def _layernorm(x):
    m = jnp.mean(x, axis=-1, keepdims=True)
    d = x - m
    v = jnp.mean(d * d, axis=-1, keepdims=True)
    return d * jax.lax.rsqrt(v + EPS)


def _kernel(x_hbm, k_hbm, v_hbm, wq_hbm, wot_hbm, w3_hbm, w4t_hbm, c_hbm, wm_hbm, o_hbm,
            x_buf, c_buf, wm_buf, wq_buf, k_buf, v_buf, wot_buf, w3_buf, w4t_buf, o_buf,
            head_buf, p_buf, gate_buf, base_buf, g_buf, sems):
    window = k_buf.shape[1]
    win = pl.ds(k_hbm.shape[2] - window, window)
    copies = {}

    def start(name, src, dst):
        copies[name] = pltpu.make_async_copy(src, dst, sems.at[len(copies)])
        copies[name].start()

    start("wm", wm_hbm, wm_buf)
    start("x", x_hbm, x_buf)
    start("c", c_hbm, c_buf)
    start("wq", wq_hbm, wq_buf)
    start("k", k_hbm.at[0, :, win, :], k_buf)
    start("v", v_hbm.at[0, :, win, :], v_buf)
    start("wo", wot_hbm, wot_buf)
    start("w3", w3_hbm, w3_buf)
    row = 0
    for i, n in enumerate((W4_MXU_ROWS,) + W4_VPU_ROWS):
        start(("w4", i), w4t_hbm.at[pl.ds(row, n)], w4t_buf.at[pl.ds(row, n)])
        row += n

    copies["wm"].wait()
    copies["x"].wait()
    copies["c"].wait()
    c = jnp.broadcast_to(c_buf[...].astype(f32), (SUB, D))
    x = jnp.broadcast_to(x_buf[0].astype(f32), (SUB, D))
    mod = jnp.dot((c * jax.nn.sigmoid(c)).astype(bf16), wm_buf[...], preferred_element_type=f32)
    sa, ca, ga, sb, cb, gb = [mod[:, i * D:(i + 1) * D] for i in range(6)]
    gate_buf[...] = gb
    h = (_layernorm(x) * (1.0 + ca) + sa).astype(bf16)

    copies["wq"].wait()
    q = jnp.dot(h, wq_buf[...], preferred_element_type=f32)
    even = jax.lax.broadcasted_iota(jnp.int32, (SUB, DH), 0) % 2 == 0
    for j in range(HKV):
        lo = 2 * j * DH
        head_buf[j] = jnp.where(even, q[:, lo:lo + DH], q[:, lo + DH:lo + 2 * DH])

    copies["k"].wait()

    def probs(j, carry):
        s = jax.lax.dot_general(head_buf[j].astype(bf16), k_buf[j], _NT,
                                preferred_element_type=f32) * (DH ** -0.5)
        p = jnp.exp(s - jnp.max(s, axis=-1, keepdims=True))
        p_buf[j] = p * (1.0 / jnp.sum(p, axis=-1, keepdims=True))
        return carry

    jax.lax.fori_loop(0, HKV, probs, None)

    copies["v"].wait()

    def values(j, carry):
        head_buf[j] = jnp.dot(p_buf[j].astype(bf16), v_buf[j], preferred_element_type=f32)
        return carry

    jax.lax.fori_loop(0, HKV, values, None)

    copies["wo"].wait()
    parts = []
    for j in range(HKV):
        o = head_buf[j]
        parts += [jnp.where(even, o, 0.0), jnp.where(even, 0.0, o)]
    o = jnp.concatenate(parts, axis=1).astype(bf16)
    a = jax.lax.dot_general(o, wot_buf[...], _NT, preferred_element_type=f32)
    x2 = x + ga * (a + pltpu.roll(a, 1, 0))
    x1 = _layernorm(x2) * (1.0 + cb) + sb
    base_buf[...] = x2 + gate_buf[...] * x1

    copies["w3"].wait()
    g = jnp.dot(_layernorm(x1).astype(bf16), w3_buf[...], preferred_element_type=f32)
    g = jax.nn.gelu(g, approximate=True).astype(bf16)
    g_buf[...] = g.astype(f32)

    def emit(lo, hi, y):
        o_buf[0, :, lo:hi] = (base_buf[0:1, lo:hi] + gate_buf[0:1, lo:hi] * y).astype(bf16)

    copies["w4", 0].wait()
    y = jax.lax.dot_general(g, w4t_buf[:W4_MXU_ROWS, :], _NT, preferred_element_type=f32)
    emit(0, W4_MXU_ROWS, y[0:1])

    def lane_partials(r):
        acc = [None, None]
        for t in range(F // LANE):
            cols = slice(t * LANE, (t + 1) * LANE)
            term = w4t_buf[r:r + SUB, cols].astype(f32) * g_buf[:, cols]
            acc[t % 2] = term if acc[t % 2] is None else acc[t % 2] + term
        return acc[0] + acc[1]

    diag = (jax.lax.broadcasted_iota(jnp.int32, (SUB, LANE), 1)
            - jax.lax.broadcasted_iota(jnp.int32, (SUB, LANE), 0))
    pending = []
    tiles = {}
    row = W4_MXU_ROWS
    for i, n in enumerate(W4_VPU_ROWS):
        copies["w4", i + 1].wait()
        pending += [(r, lane_partials(r)) for r in range(row, row + n, SUB)]
        row += n
        if row < D and i >= len(W4_VPU_ROWS) - W4_VPU_DEFERRED:
            continue
        for r, partial in pending:
            tiles[r // LANE] = jnp.where(diag == r % LANE, jnp.sum(partial, axis=-1, keepdims=True),
                                         tiles.get(r // LANE, 0.0))
        pending = []
        for t in sorted(tiles):
            lo, hi = t * LANE, min((t + 1) * LANE, D)
            if hi <= row:
                emit(lo, hi, jnp.sum(tiles.pop(t), axis=0, keepdims=True)[:, :hi - lo])

    out = pltpu.make_async_copy(o_buf, o_hbm, sems.at[len(copies)])
    out.start()
    out.wait()


@jax.jit
def pallas_adaLN_cond__sliding_block_cached__mixer_s_mlp__decode_kernel(
    A_x: jax.Array,
    A_k_cache: jax.Array,
    A_v_cache: jax.Array,
    A_wq: jax.Array,
    A_wo: jax.Array,
    B_x: jax.Array,
    B_w1: jax.Array,
    B_w2: jax.Array,
    B_w3: jax.Array,
    B_w4: jax.Array,
    c: jax.Array,
    w_mod: jax.Array,
):
    assert A_x.shape == (1, 1, D) and A_k_cache.shape[:2] == (1, HKV)
    assert W4_MXU_ROWS + sum(W4_VPU_ROWS) == D
    window = min(4096, max(256, A_k_cache.shape[2] // 4))
    hbm = pl.BlockSpec(memory_space=pltpu.HBM)
    return pl.pallas_call(
        _kernel,
        out_shape=pltpu.HBM(A_x.shape, bf16),
        in_specs=[hbm] * 9,
        out_specs=hbm,
        scratch_shapes=[
            pltpu.VMEM((1, 1, D), bf16),
            pltpu.VMEM((1, D), bf16),
            pltpu.VMEM((D, 6 * D), bf16),
            pltpu.VMEM((D, HQ * DH), bf16),
            pltpu.VMEM((HKV, window, DH), bf16),
            pltpu.VMEM((HKV, window, DH), bf16),
            pltpu.VMEM((D, HQ * DH), bf16),
            pltpu.VMEM((D, F), bf16),
            pltpu.VMEM((D, F), bf16),
            pltpu.VMEM((1, 1, D), bf16),
            pltpu.VMEM((HKV, SUB, DH), f32),
            pltpu.VMEM((HKV, SUB, window), f32),
            pltpu.VMEM((SUB, D), f32),
            pltpu.VMEM((SUB, D), f32),
            pltpu.VMEM((SUB, F), f32),
            pltpu.SemaphoreType.DMA((10 + len(W4_VPU_ROWS),)),
        ],
        compiler_params=pltpu.CompilerParams(
            vmem_limit_bytes=64 * 2**20,
            disable_bounds_checks=True,
            disable_semaphore_checks=True,
        ),
    )(A_x, A_k_cache, A_v_cache, A_wq, A_wo.T, B_w3, B_w4.T, c, w_mod)
```

```python
import jax
import jax.numpy as jnp
import jax.experimental.pallas as pl
import jax.experimental.pallas.tpu as pltpu

D = 448
F = 1792
HQ = 16
HKV = 8
DH = 256
EPS = 1e-5
SUB = 8
LANE = 128

W4_MXU_ROWS = 256
W4_VPU_ROWS = (96, 56, 32, 8)
W4_VPU_DEFERRED = 2

_NT = (((1,), (1,)), ((), ()))
bf16 = jnp.bfloat16
f32 = jnp.float32


def _layernorm(x):
    m = jnp.mean(x, axis=-1, keepdims=True)
    d = x - m
    v = jnp.mean(d * d, axis=-1, keepdims=True)
    return d * jax.lax.rsqrt(v + EPS)


def _kernel(x_hbm, k_hbm, v_hbm, wq_hbm, wot_hbm, w3_hbm, w4t_hbm, c_hbm, wm_hbm, o_ref,
            x_buf, c_buf, wm_buf, wq_buf, k_buf, v_buf, wot_buf, w3_buf, w4t_buf,
            head_buf, p_buf, gate_buf, base_buf, g_buf, sems):
    window = k_buf.shape[1]
    win = pl.ds(k_hbm.shape[2] - window, window)
    copies = {}

    def start(name, src, dst):
        copies[name] = pltpu.make_async_copy(src, dst, sems.at[len(copies)])
        copies[name].start()

    start("wm", wm_hbm, wm_buf)
    start("x", x_hbm, x_buf)
    start("c", c_hbm, c_buf)
    start("wq", wq_hbm, wq_buf)
    start("k", k_hbm.at[0, :, win, :], k_buf)
    start("v", v_hbm.at[0, :, win, :], v_buf)
    start("wo", wot_hbm, wot_buf)
    start("w3", w3_hbm, w3_buf)
    row = 0
    for i, n in enumerate((W4_MXU_ROWS,) + W4_VPU_ROWS):
        start(("w4", i), w4t_hbm.at[pl.ds(row, n)], w4t_buf.at[pl.ds(row, n)])
        row += n

    copies["wm"].wait()
    copies["x"].wait()
    copies["c"].wait()
    c = jnp.broadcast_to(c_buf[...].astype(f32), (SUB, D))
    x = jnp.broadcast_to(x_buf[0].astype(f32), (SUB, D))
    mod = jnp.dot((c * jax.nn.sigmoid(c)).astype(bf16), wm_buf[...], preferred_element_type=f32)
    sa, ca, ga, sb, cb, gb = [mod[:, i * D:(i + 1) * D] for i in range(6)]
    gate_buf[...] = gb
    h = (_layernorm(x) * (1.0 + ca) + sa).astype(bf16)

    copies["wq"].wait()
    q = jnp.dot(h, wq_buf[...], preferred_element_type=f32)
    even = jax.lax.broadcasted_iota(jnp.int32, (SUB, DH), 0) % 2 == 0
    for j in range(HKV):
        lo = 2 * j * DH
        head_buf[j] = jnp.where(even, q[:, lo:lo + DH], q[:, lo + DH:lo + 2 * DH])

    copies["k"].wait()

    def probs(j, carry):
        s = jax.lax.dot_general(head_buf[j].astype(bf16), k_buf[j], _NT,
                                preferred_element_type=f32) * (DH ** -0.5)
        p = jnp.exp(s - jnp.max(s, axis=-1, keepdims=True))
        p_buf[j] = p * (1.0 / jnp.sum(p, axis=-1, keepdims=True))
        return carry

    jax.lax.fori_loop(0, HKV, probs, None)

    copies["v"].wait()

    def values(j, carry):
        head_buf[j] = jnp.dot(p_buf[j].astype(bf16), v_buf[j], preferred_element_type=f32)
        return carry

    jax.lax.fori_loop(0, HKV, values, None)

    copies["wo"].wait()
    parts = []
    for j in range(HKV):
        o = head_buf[j]
        parts += [jnp.where(even, o, 0.0), jnp.where(even, 0.0, o)]
    o = jnp.concatenate(parts, axis=1).astype(bf16)
    a = jax.lax.dot_general(o, wot_buf[...], _NT, preferred_element_type=f32)
    x2 = x + ga * (a + pltpu.roll(a, 1, 0))
    x1 = _layernorm(x2) * (1.0 + cb) + sb
    base_buf[...] = x2 + gate_buf[...] * x1

    copies["w3"].wait()
    g = jnp.dot(_layernorm(x1).astype(bf16), w3_buf[...], preferred_element_type=f32)
    g = jax.nn.gelu(g, approximate=True).astype(bf16)
    g_buf[...] = g.astype(f32)

    def emit(lo, hi, y):
        o_ref[0, :, lo:hi] = (base_buf[0:1, lo:hi] + gate_buf[0:1, lo:hi] * y).astype(bf16)

    copies["w4", 0].wait()
    y = jax.lax.dot_general(g, w4t_buf[:W4_MXU_ROWS, :], _NT, preferred_element_type=f32)
    emit(0, W4_MXU_ROWS, y[0:1])

    def lane_partials(r):
        acc = [None, None]
        for t in range(F // LANE):
            cols = slice(t * LANE, (t + 1) * LANE)
            term = w4t_buf[r:r + SUB, cols].astype(f32) * g_buf[:, cols]
            acc[t % 2] = term if acc[t % 2] is None else acc[t % 2] + term
        return acc[0] + acc[1]

    diag = (jax.lax.broadcasted_iota(jnp.int32, (SUB, LANE), 1)
            - jax.lax.broadcasted_iota(jnp.int32, (SUB, LANE), 0))
    pending = []
    tiles = {}
    row = W4_MXU_ROWS
    for i, n in enumerate(W4_VPU_ROWS):
        copies["w4", i + 1].wait()
        pending += [(r, lane_partials(r)) for r in range(row, row + n, SUB)]
        row += n
        if row < D and i >= len(W4_VPU_ROWS) - W4_VPU_DEFERRED:
            continue
        for r, partial in pending:
            tiles[r // LANE] = jnp.where(diag == r % LANE, jnp.sum(partial, axis=-1, keepdims=True),
                                         tiles.get(r // LANE, 0.0))
        pending = []
        for t in sorted(tiles):
            lo, hi = t * LANE, min((t + 1) * LANE, D)
            if hi <= row:
                emit(lo, hi, jnp.sum(tiles.pop(t), axis=0, keepdims=True)[:, :hi - lo])


@jax.jit
def pallas_adaLN_cond__sliding_block_cached__mixer_s_mlp__decode_kernel(
    A_x: jax.Array,
    A_k_cache: jax.Array,
    A_v_cache: jax.Array,
    A_wq: jax.Array,
    A_wo: jax.Array,
    B_x: jax.Array,
    B_w1: jax.Array,
    B_w2: jax.Array,
    B_w3: jax.Array,
    B_w4: jax.Array,
    c: jax.Array,
    w_mod: jax.Array,
):
    assert A_x.shape == (1, 1, D) and A_k_cache.shape[:2] == (1, HKV)
    assert W4_MXU_ROWS + sum(W4_VPU_ROWS) == D
    window = min(4096, max(256, A_k_cache.shape[2] // 4))
    hbm = pl.BlockSpec(memory_space=pltpu.HBM)
    return pl.pallas_call(
        _kernel,
        out_shape=jax.ShapeDtypeStruct(A_x.shape, bf16),
        in_specs=[hbm] * 9,
        scratch_shapes=[
            pltpu.VMEM((1, 1, D), bf16),
            pltpu.VMEM((1, D), bf16),
            pltpu.VMEM((D, 6 * D), bf16),
            pltpu.VMEM((D, HQ * DH), bf16),
            pltpu.VMEM((HKV, window, DH), bf16),
            pltpu.VMEM((HKV, window, DH), bf16),
            pltpu.VMEM((D, HQ * DH), bf16),
            pltpu.VMEM((D, F), bf16),
            pltpu.VMEM((D, F), bf16),
            pltpu.VMEM((HKV, SUB, DH), f32),
            pltpu.VMEM((HKV, SUB, window), f32),
            pltpu.VMEM((SUB, D), f32),
            pltpu.VMEM((SUB, D), f32),
            pltpu.VMEM((SUB, F), f32),
            pltpu.SemaphoreType.DMA((9 + len(W4_VPU_ROWS),)),
        ],
        compiler_params=pltpu.CompilerParams(
            vmem_limit_bytes=64 * 2**20,
            disable_bounds_checks=True,
            disable_semaphore_checks=True,
        ),
    )(A_x, A_k_cache, A_v_cache, A_wq, A_wo.T, B_w3, B_w4.T, c, w_mod)
```
